```python
import os as _os
_os.environ.setdefault("JAX_PLATFORMS", "cpu")
import jax
import jax.numpy as jnp

def _softmax(x, axis=-1):
    return jax.nn.softmax(x, axis=axis)
def _gelu(x):
    return jax.nn.gelu(x, approximate=True)
def _silu(x):
    return jax.nn.silu(x)
def _sigmoid(x):
    return jax.nn.sigmoid(x)
def _layernorm(x, axis=-1, eps=1e-5):
    m = jnp.mean(x, axis=axis, keepdims=True)
    v = jnp.var(x, axis=axis, keepdims=True)
    return (x - m) / jnp.sqrt(v + eps)
def _scatter_add(tgt, idx, src, axis=0):
    return tgt.at[idx].add(src)
def _segment_sum(src, seg, n):
    return jax.ops.segment_sum(src, seg, n)
class _Rng:
    def __init__(self, key):
        self._k = key
    def _next(self):
        self._k, sub = jax.random.split(self._k)
        return sub
    def normal(self, shape):
        return jax.random.normal(self._next(), shape, dtype=jnp.bfloat16)
    def randint(self, lo, hi, shape):
        return jax.random.randint(self._next(), shape, lo, hi, dtype=jnp.int32)
    def uniform(self, shape, lo=0.0, hi=1.0):
        return jax.random.uniform(self._next(), shape, jnp.bfloat16, lo, hi)
    def permutation(self, n):
        return jax.random.permutation(self._next(), n)


kernel_name = 'gated_mix__mha_block__mixer_s_mlp__prompt'

def setup_inputs():
    _rng = _Rng(jax.random.key(int.from_bytes(__import__("os").urandom(4), "little")))
    _w = (lambda a: (lambda t: t.astype(jnp.bfloat16) if jnp.issubdtype(t.dtype, jnp.floating) else t)(jnp.asarray(a)))
    def _A_setup():
        B, S, D, H = 1, 2048, 512, 32
        return {
            "x": _w((lambda *s: _rng.normal(s) * 0.05)(B, S, D)),
            "wqkv": _w((lambda *s: _rng.normal(s) * 0.8)(D, 3 * D)),
            "wo": _w((lambda *s: _rng.normal(s) * 0.05)(D, D)),
        }
    _A_in = _A_setup()

    def _B_setup():
        B, S, D, F = 1, 2048, 512, 1792
        return {
            "x":  _w((lambda *s: _rng.normal(s) * 0.05)(B, S, D)),
            "w1": _w((lambda *s: _rng.normal(s) * 0.2)(D, D) * (D ** -0.5)),
            "w2": _w((lambda *s: _rng.normal(s) * 0.2)(D, D) * (D ** -0.5)),
            "w3": _w((lambda *s: _rng.normal(s) * 0.2)(D, F) * (D ** -0.5)),
            "w4": _w((lambda *s: _rng.normal(s) * 0.2)(F, D) * (F ** -0.5)),
        }
    _B_in = _B_setup()

    return {
        "A_x": _A_in["x"],
        "A_wqkv": _A_in["wqkv"],
        "A_wo": _A_in["wo"],
        "B_x": _B_in["x"],
        "B_w1": _B_in["w1"],
        "B_w2": _B_in["w2"],
        "B_w3": _B_in["w3"],
        "B_w4": _B_in["w4"],
        "gate_w": _w((lambda *s: _rng.normal(s) * 0.05)(512) * 16.0),
    }

def reference(A_x, A_wqkv, A_wo, B_x, B_w1, B_w2, B_w3, B_w4, gate_w):
    def _A_ref(x, wqkv, wo):
        B, S, D = x.shape
        H = 32
        Dh = D // H
        qkv = (lambda x, *d: x.transpose(*d))((x @ wqkv).reshape(B, S, 3, H, Dh), 2, 0, 3, 1, 4)
        q, k, v = qkv[0], qkv[1], qkv[2]
        scores = jnp.einsum("bhqd,bhkd->bhqk", q, k) * (Dh ** -0.5)
        p = _softmax(scores, axis=-1)
        o = jnp.einsum("bhqk,bhkd->bhqd", p, v)
        return (lambda x, *d: x.transpose(*d))(o, 0, 2, 1, 3).reshape(B, S, D) @ wo

    def _B_ref(x, w1, w2, w3, w4):
        B, S, D = x.shape
        h = _gelu(_layernorm(x, axis=-1) @ w1)
        c = D // 4
        g0 = jnp.pad(h[:, :, 0*c:1*c], ((0, 0), (1, 0), (0, 0)))[:, :S, :]
        g1 = jnp.pad(h[:, :, 1*c:2*c], ((0, 0), (0, 1), (0, 0)))[:, 1:, :]
        g2 = jnp.pad(h[:, :, 2*c:3*c], ((0, 0), (2, 0), (0, 0)))[:, :S, :]
        g3 = jnp.pad(h[:, :, 3*c:   ], ((0, 0), (0, 2), (0, 0)))[:, 2:, :]
        hs = jnp.concatenate([g0, g1, g2, g3], axis=-1) @ w2
        x1 = x + hs
        h2 = _gelu(_layernorm(x1, axis=-1) @ w3) @ w4
        return x1 + h2

    x = A_x
    g = _sigmoid((x * gate_w).sum(-1, keepdims=True))
    a = _A_ref(x, A_wqkv, A_wo)
    b = _B_ref(x, B_w1, B_w2, B_w3, B_w4)
    return g * a + (1 - g) * b
```

```python
import functools

import jax
import jax.numpy as jnp
import numpy as np
from jax import lax
from jax.experimental import pallas as pl
from jax.experimental.pallas import tpu as pltpu

F32 = jnp.float32
BF16 = jnp.bfloat16

S, D, H, DH, FF = 2048, 512, 32, 16, 1792
EPS = 1e-5
Q_SCALE = float(DH ** -0.5 * np.log2(np.e))
GELU_C1 = float(np.sqrt(2.0 / np.pi))
GELU_C2 = float(np.sqrt(2.0 / np.pi) * 0.044715)
L_MIN, L_MAX, F32_MAX = 1.0, float(2.0 ** 100), float(np.finfo(np.float32).max)

R1 = (256, 256, 512, 512, 512)
BQ = 512
BK = 128
NQ = S // BQ
LAG = 2
SLAB = 16
VK = (0,) + (16,) * 15
J0 = 4
G0 = 2
QSPAN = 8
R3 = 256
PAD = 8

ORDER_A = (3, 6, 5, 4, 2, 7, 1)
ORDER_B = (2, 4, 1, 7, 5, 3, 6)

NN = (((1,), (0,)), ((), ()))
NT = (((1,), (1,)), ((), ()))
TN = (((0,), (0,)), ((), ()))


def _dot(a, b, dims=NN):
    return lax.dot_general(a, b, dims, preferred_element_type=F32)


def _gelu(x):
    hx = 0.5 * x
    return hx + hx * jnp.tanh(x * (GELU_C1 + GELU_C2 * (x * x)))


def _layernorm(x):
    d = x - jnp.mean(x, axis=-1, keepdims=True)
    return d * lax.rsqrt(jnp.mean(d * d, axis=-1, keepdims=True) + EPS)


def _quads(a):
    m, n = a.shape[0] // 2, a.shape[1] // 2
    return a[:m, :n], a[:m, n:], a[m:, :n], a[m:, n:]


def _strassen_rhs(w_ref, sums_ref, start, rows):
    k, n = w_ref.shape[0] // 2, w_ref.shape[1] // 2
    for r in range(0, rows, SLAB):
        top, bot = pl.ds(start + r, SLAB), pl.ds(start + k + r, SLAB)
        b11, b12 = w_ref[top, :n].astype(F32), w_ref[top, n:].astype(F32)
        b21, b22 = w_ref[bot, :n].astype(F32), w_ref[bot, n:].astype(F32)
        for i, b in enumerate((b11 + b22, b12 - b22, b21 - b11, b11 + b12, b21 + b22)):
            sums_ref[i, top, :] = b.astype(BF16)


def _strassen(a, w_ref, sums_ref, order):
    a11, a12, a21, a22 = a
    k, n = w_ref.shape[0] // 2, w_ref.shape[1] // 2
    product = {
        1: lambda: _dot((a11 + a22).astype(BF16), sums_ref[0]),
        2: lambda: _dot((a21 + a22).astype(BF16), w_ref[:k, :n]),
        3: lambda: _dot(a11.astype(BF16), sums_ref[1]),
        4: lambda: _dot(a22.astype(BF16), sums_ref[2]),
        5: lambda: _dot((a11 + a12).astype(BF16), w_ref[k:, n:]),
        6: lambda: _dot((a21 - a11).astype(BF16), sums_ref[3]),
        7: lambda: _dot((a12 - a22).astype(BF16), sums_ref[4]),
    }
    m = {i: product[i]() for i in order}
    c11 = (m[1] + m[4]) + (m[7] - m[5])
    c12 = m[3] + m[5]
    c21 = m[2] + m[4]
    c22 = (m[1] - m[2]) + (m[3] + m[6])
    return c11, c12, c21, c22


def _join(c11, c12, c21, c22):
    return jnp.concatenate([jnp.concatenate([c11, c12], axis=1),
                            jnp.concatenate([c21, c22], axis=1)], axis=0)


def _kernel(xa_hbm, wqkv_hbm, wo_hbm, w1_hbm, w2_hbm, w3_hbm, w4_hbm, gw_hbm,
            out_hbm,
            xa, wqkv, wo, w1, w2, w3, w4, gw, out,
            wq_t, k_s, qt_s, vt_s, ot_s, p_c, acc_c, l_c, h_s, w3_s, w4_s, w1_s, wv_s,
            sem_a, sem_w, sem_o):
    n3 = S // R3
    starts = [int(v) for v in np.cumsum((0,) + R1)]
    g = D // 4
    wv = wqkv.at[:, 2 * D:3 * D]

    def w_copy(i):
        cols = pl.ds(i * D, D)
        return pltpu.make_async_copy(wqkv_hbm.at[:, cols], wqkv.at[:, cols], sem_w.at[i])

    def xa_copy(r):
        rows = pl.ds(starts[r], R1[r])
        return pltpu.make_async_copy(xa_hbm.at[rows, :], xa.at[rows, :], sem_a.at[r])

    w1_copy = pltpu.make_async_copy(w1_hbm, w1, sem_w.at[3])
    late = [pltpu.make_async_copy(src, dst, sem_w.at[4 + i]) for i, (src, dst) in enumerate(
        ((w3_hbm, w3), (w4_hbm, w4), (w2_hbm, w2), (wo_hbm, wo), (gw_hbm, gw)))]
    w_copy(1).start()
    xa_copy(0).start()
    w_copy(0).start()
    for i in range(4):
        h_s[i, 0:PAD, :] = jnp.zeros((PAD, g), F32)
        h_s[i, PAD + S:2 * PAD + S, :] = jnp.zeros((PAD, g), F32)
    p_c[...] = jnp.zeros_like(p_c)
    acc_c[...] = jnp.zeros_like(acc_c)
    l_c[...] = jnp.full(l_c.shape, 0.125, F32)
    w_copy(1).wait()
    xa_copy(0).wait()
    for c in (w1_copy, w_copy(2), xa_copy(1)):
        c.start()

    for r in range(len(R1)):
        rows = pl.ds(starts[r], R1[r])
        if r == 1:
            xa_copy(1).wait()
            for c in [xa_copy(i) for i in range(2, len(R1))] + late:
                c.start()
        if r == 2:
            for i in range(2, len(R1)):
                xa_copy(i).wait()
        x = xa[rows, :]
        xn = _layernorm(x.astype(F32))
        k = _dot(x, wqkv[:, D:2 * D]).astype(BF16)
        for h in range(H):
            k_s[h, rows, :] = k[:, h * DH:(h + 1) * DH]
        if r == 0:
            w_copy(0).wait()
            wq_t[...] = wqkv[:, 0:D].astype(F32).T.astype(BF16)
        qt_s[:, rows] = (_dot(wq_t[...], x, NT) * Q_SCALE).astype(BF16)
        if r == 0:
            w1_copy.wait()
            _strassen_rhs(w1, w1_s, 0, D // 2)
        hh = _gelu(_join(*_strassen(_quads(xn), w1, w1_s, ORDER_A)))
        for i in range(4):
            h_s[i, pl.ds(PAD + starts[r], R1[r]), :] = hh[:, i * g:(i + 1) * g]
        if r == 0:
            w_copy(2).wait()
            _strassen_rhs(wv, wv_s, 0, D // 2)
        v = _join(*_strassen(_quads(x.astype(F32)), wv, wv_s, ORDER_A))
        vt_s[:, rows] = v.astype(BF16).T

    for c in late:
        c.wait()

    nk = S // BK
    steps = [(j, q) for q in range(NQ) for j in range(nk)]
    nt = len(steps)

    def features(h):
        return pl.ds(pl.multiple_of(h * DH, DH), DH)

    def finish(feat, q, acc, l8, bad):
        l = jnp.sum(l8, axis=0, keepdims=True)
        o = acc * (1.0 / l)
        ot_s[feat, q * BQ:(q + 1) * BQ] = o.astype(BF16)
        ok = (jnp.abs(o) <= F32_MAX) & (l >= L_MIN) & (l <= L_MAX)
        f = jnp.where(ok, 0.0, 1.0)
        f = jnp.maximum(f[:8], f[8:])
        return functools.reduce(jnp.maximum, [f[:, c:c + 128] for c in range(0, BQ, 128)], bad)

    def tail(feat, bad):
        acc = acc_c[...]
        for t in range(LAG):
            j = nk - LAG + t
            acc = acc + _dot(vt_s[feat, j * BK:(j + 1) * BK], p_c[t])
            if t == LAG - 1:
                bad = finish(feat, NQ - 1, acc, l_c[...], bad)
            yield bad

    def attend(h, bad):
        feat = features(h)
        previous = tail(features(jnp.maximum(h - 1, 0)), bad)
        acc, l8, ps = [None] * NQ, [None] * NQ, {}

        def key_cols(j, gate=None):
            keys = k_s[h, (j + 1) * BK - VK[j]:(j + 1) * BK, :].astype(F32)
            if gate is not None:
                keys = keys + gate
            return [jnp.broadcast_to(keys[:, d:d + 1], (VK[j], 128)) for d in range(DH)]

        def query_rows(q, gate=None):
            queries = qt_s[feat, q * BQ:(q + 1) * BQ].astype(F32)
            if gate is not None:
                queries = queries + gate
            return [jnp.broadcast_to(queries[d:d + 1], (8, BQ)) for d in range(DH)]

        kb = {j: key_cols(j) for j in range(J0) if VK[j]}
        qb = {q: query_rows(q) for q in range(1, NQ)}
        for t, (j, q) in enumerate(steps):
            vk = VK[j] if t >= J0 else 0
            s = _dot(k_s[h, j * BK:(j + 1) * BK - vk, :], qt_s[feat, q * BQ:(q + 1) * BQ])
            if vk:
                sv = None
                for d in range(DH):
                    kd = jnp.concatenate([kb[j][d]] * (BQ // 128), axis=1)
                    m = kd.reshape(vk // 8, 8, BQ) * qb[q][d][None]
                    sv = m if sv is None else sv + m
                s = jnp.concatenate([s, sv.reshape(vk, BQ)], axis=0)
            p = jnp.exp2(s)
            if l8[q] is None:
                ls = p.reshape(BK // 8, 8, BQ).sum(0)
            else:
                ls = functools.reduce(jnp.add, [p[r:r + 8] for r in range(0, BK, 8)], l8[q])
            early = [x[r:r + 8] for jj in range(J0) if VK[jj] and t == jj * (J0 - G0) // J0
                     for x in kb[jj] for r in range(0, VK[jj], 8)]
            if early:
                z = functools.reduce(jnp.add, early) * 0.0
                ls = ls + jnp.concatenate([z] * (BQ // 128), axis=1)
            if q < NQ - 1 and -1 <= j - nk + QSPAN < QSPAN - 1:
                e, per = j - nk + QSPAN + 1, DH // QSPAN
                for d in range(e * per, (e + 1) * per):
                    ls = ls + qb[q + 1][d] * 0.0
            l8[q] = ls
            if J0 <= t + G0 < nk and VK[t + G0]:
                gate = jnp.concatenate([ls[:, 0:DH] * 0.0] * (VK[t + G0] // 8), axis=0)
                kb[t + G0] = key_cols(t + G0, gate)
            if t == J0 - G0:
                qb[0] = query_rows(0, ls[0:1] * 0.0)
            if t >= nt - LAG:
                p_c[t - (nt - LAG)] = p.astype(BF16)
            else:
                ps[t] = p.astype(BF16)
            if t < LAG:
                bad = next(previous)
                continue
            j2, q2 = steps[t - LAG]
            d = _dot(vt_s[feat, j2 * BK:(j2 + 1) * BK], ps.pop(t - LAG))
            acc[q2] = d if acc[q2] is None else acc[q2] + d
            if j2 == nk - 1:
                bad = finish(feat, q2, acc[q2], l8[q2], bad)
        acc_c[...] = acc[NQ - 1]
        l_c[...] = l8[NQ - 1]
        return bad

    def attend_and_sum(h, bad):
        bad = attend(h, bad)
        for w, sums in ((w3, w3_s), (w4, w4_s)):
            half = w.shape[0] // 2
            slab = pl.cdiv(half, H * SLAB) * SLAB
            start = pl.multiple_of(jnp.minimum(h * slab, half - slab), SLAB)
            _strassen_rhs(w, sums, start, slab)
        return bad

    bad = lax.fori_loop(0, H, attend_and_sum, jnp.zeros((8, 128), F32))
    for bad in tail(features(H - 1), bad):
        pass

    @pl.when(jnp.max(bad) > 0.0)
    def _attention_with_true_max():
        sq, sk = 256, 256

        def block(it, _):
            h = it // (S // sq)
            feat = features(h)
            cols = pl.ds(pl.multiple_of((it % (S // sq)) * sq, sq), sq)
            qt = qt_s[feat, cols]

            def tile(j, carry):
                m, l, acc = carry
                keys = pl.ds(pl.multiple_of(j * sk, sk), sk)
                s = _dot(k_s[h, keys, :], qt)
                m_new = jnp.maximum(m, jnp.max(s, axis=0, keepdims=True))
                alpha = jnp.exp2(m - m_new)
                p = jnp.exp2(s - m_new)
                l = alpha * l + jnp.sum(p, axis=0, keepdims=True)
                acc = alpha * acc + _dot(vt_s[feat, keys], p.astype(BF16))
                return m_new, l, acc

            init = (jnp.full((1, sq), -F32_MAX, F32), jnp.zeros((1, sq), F32),
                    jnp.zeros((DH, sq), F32))
            _, l, acc = lax.fori_loop(0, S // sk, tile, init)
            ot_s[feat, cols] = (acc * (1.0 / l)).astype(BF16)
            return 0

        lax.fori_loop(0, H * (S // sq), block, 0)

    def out_copy(r):
        rows = pl.ds(r * R3, R3)
        return pltpu.make_async_copy(out.at[rows, :], out_hbm.at[rows, :], sem_o.at[r])

    def mix(r, _):
        r0 = pl.multiple_of(r * R3, R3)
        rows = pl.ds(r0, R3)
        hs = jnp.concatenate(
            [h_s[i, pl.ds(PAD + r0 - shift, R3), :]
             for i, shift in enumerate((1, -1, 2, -2))], axis=1)
        x = xa[rows, :].astype(F32)
        x1 = x + _dot(hs.astype(BF16), w2[...])
        xn = _layernorm(x1)
        gate = jax.nn.sigmoid(
            jnp.sum(x * gw[...].astype(F32).reshape(1, D), axis=-1, keepdims=True))
        a0 = _dot(ot_s[:, rows], wo[:, :D // 2], TN)
        h2 = [_gelu(c) for c in _strassen(_quads(xn), w3, w3_s, ORDER_B)]
        a1 = _dot(ot_s[:, rows], wo[:, D // 2:], TN)
        b = x1 + _join(*_strassen(h2, w4, w4_s, ORDER_A))
        a = jnp.concatenate([a0, a1], axis=1)
        out[rows, :] = (gate * a + (1.0 - gate) * b).astype(BF16)
        out_copy(r).start()
        return 0

    lax.fori_loop(0, n3, mix, 0)
    for r in range(n3):
        out_copy(r).wait()


@jax.jit
def pallas_gated_mix__mha_block__mixer_s_mlp__prompt_kernel(
    A_x: jax.Array,
    A_wqkv: jax.Array,
    A_wo: jax.Array,
    B_x: jax.Array,
    B_w1: jax.Array,
    B_w2: jax.Array,
    B_w3: jax.Array,
    B_w4: jax.Array,
    gate_w: jax.Array,
):
    vmem = pltpu.VMEM
    hbm = pl.BlockSpec(memory_space=pl.ANY)
    out = pl.pallas_call(
        _kernel,
        out_shape=jax.ShapeDtypeStruct((S, D), BF16),
        in_specs=[hbm] * 8,
        out_specs=hbm,
        scratch_shapes=[
            vmem((S, D), BF16), vmem((D, 3 * D), BF16), vmem((D, D), BF16),
            vmem((D, D), BF16), vmem((D, D), BF16),
            vmem((D, FF), BF16), vmem((FF, D), BF16), vmem((D,), BF16),
            vmem((S, D), BF16),
            vmem((D, D), BF16),
            vmem((H, S, DH), BF16),
            vmem((D, S), BF16), vmem((D, S), BF16), vmem((D, S), BF16),
            vmem((LAG, BK, BQ), BF16), vmem((DH, BQ), F32), vmem((8, BQ), F32),
            vmem((4, S + 2 * PAD, D // 4), F32),
            vmem((5, D // 2, FF // 2), BF16), vmem((5, FF // 2, D // 2), BF16),
            *[vmem((5, D // 2, D // 2), BF16)] * 2,
            pltpu.SemaphoreType.DMA((len(R1),)),
            pltpu.SemaphoreType.DMA((9,)),
            pltpu.SemaphoreType.DMA((S // R3,)),
        ],
        compiler_params=pltpu.CompilerParams(vmem_limit_bytes=110 * 1024 * 1024),
    )(A_x.reshape(S, D), A_wqkv, A_wo, B_w1, B_w2, B_w3, B_w4, gate_w)
    return out.reshape(1, S, D)
```
